```python
import os as _os
_os.environ.setdefault("JAX_PLATFORMS", "cpu")
import jax
import jax.numpy as jnp

def _softmax(x, axis=-1):
    return jax.nn.softmax(x, axis=axis)
def _gelu(x):
    return jax.nn.gelu(x, approximate=True)
def _silu(x):
    return jax.nn.silu(x)
def _sigmoid(x):
    return jax.nn.sigmoid(x)
def _layernorm(x, axis=-1, eps=1e-5):
    m = jnp.mean(x, axis=axis, keepdims=True)
    v = jnp.var(x, axis=axis, keepdims=True)
    return (x - m) / jnp.sqrt(v + eps)
def _scatter_add(tgt, idx, src, axis=0):
    return tgt.at[idx].add(src)
def _segment_sum(src, seg, n):
    return jax.ops.segment_sum(src, seg, n)
class _Rng:
    def __init__(self, key):
        self._k = key
    def _next(self):
        self._k, sub = jax.random.split(self._k)
        return sub
    def normal(self, shape):
        return jax.random.normal(self._next(), shape, dtype=jnp.bfloat16)
    def randint(self, lo, hi, shape):
        return jax.random.randint(self._next(), shape, lo, hi, dtype=jnp.int32)
    def uniform(self, shape, lo=0.0, hi=1.0):
        return jax.random.uniform(self._next(), shape, jnp.bfloat16, lo, hi)
    def permutation(self, n):
        return jax.random.permutation(self._next(), n)


kernel_name = 'sequential_preLN__softmax_full_mha__geglu_ffn__prompt'

def setup_inputs():
    _rng = _Rng(jax.random.key(int.from_bytes(__import__("os").urandom(4), "little")))
    _w = (lambda a: (lambda t: t.astype(jnp.bfloat16) if jnp.issubdtype(t.dtype, jnp.floating) else t)(jnp.asarray(a)))
    def _A_setup():
        B, S, D = 1, 2048, 512
        return {
            "x": _w((lambda *s: _rng.normal(s) * 0.05)(B, S, D)),
            "wqkv": _w((lambda *s: _rng.normal(s) * 0.05)(D, 3 * D)),
            "wo": _w((lambda *s: _rng.normal(s) * 0.05)(D, D)),
        }
    _A_in = _A_setup()

    def _B_setup():
        B, S, D, F = 1, 2048, 512, 1376
        return {
            "x": _w((lambda *s: _rng.normal(s) * 0.05)(B, S, D)),
            "w_gate": _w((lambda *s: _rng.normal(s) * 0.05)(D, F)),
            "w_up": _w((lambda *s: _rng.normal(s) * 0.05)(D, F)),
            "w_down": _w((lambda *s: _rng.normal(s) * 0.05)(F, D)),
        }
    _B_in = _B_setup()

    return {
        "A_x": _A_in["x"],
        "A_wqkv": _A_in["wqkv"],
        "A_wo": _A_in["wo"],
        "B_x": _B_in["x"],
        "B_w_gate": _B_in["w_gate"],
        "B_w_up": _B_in["w_up"],
        "B_w_down": _B_in["w_down"],
    }

def reference(A_x, A_wqkv, A_wo, B_x, B_w_gate, B_w_up, B_w_down):
    def _A_ref(x, wqkv, wo):
        B, S, D = x.shape
        H = 32; Dh = D // H
        qkv = (lambda x, *d: x.transpose(*d))((x @ wqkv).reshape(B, S, 3, H, Dh), 2, 0, 3, 1, 4)
        q, k, v = qkv[0], qkv[1], qkv[2]
        scale = Dh ** -0.5
        scores = jnp.einsum("bhqd,bhkd->bhqk", q, k) * scale
        p = _softmax(scores, axis=-1)
        o = jnp.einsum("bhqk,bhkd->bhqd", p, v)
        return (lambda x, *d: x.transpose(*d))(o, 0, 2, 1, 3).reshape(B, S, D) @ wo

    def _B_ref(x, w_gate, w_up, w_down):
        return (_gelu(x @ w_gate) * (x @ w_up)) @ w_down

    x = A_x
    h = x + _A_ref(_layernorm(x, axis=-1), A_wqkv, A_wo)
    h2 = h + _B_ref(_layernorm(h, axis=-1), B_w_gate, B_w_up, B_w_down)
    return h2
```

```python
import functools
import math

import jax
import jax.numpy as jnp
from jax import lax
import jax.experimental.pallas as pl
import jax.experimental.pallas.tpu as pltpu

S, D, H, DH, F = 2048, 512, 32, 16, 1376
EPS = 1e-5
QSCALE = (DH ** -0.5) * math.log2(math.e)
F32, BF16, U32 = jnp.float32, jnp.bfloat16, jnp.uint32


def _ln(x):
    m = jnp.mean(x, axis=-1, keepdims=True)
    xc = x - m
    v = jnp.mean(xc * xc, axis=-1, keepdims=True)
    return xc * lax.rsqrt(v + EPS)


def _gelu_tanh(x):
    c = math.sqrt(2.0 / math.pi)
    return 0.5 * x * (1.0 + jnp.tanh(c * (x + 0.044715 * (x * x * x))))


def _pk(x):
    return pltpu.bitcast(x, U32)


def _up(x):
    return pltpu.bitcast(x, BF16)


def make(TQ=512, TM=512, UN=6, DELAY=2, FENCE=2, P1=True, P2=True, P3=True, TP1=512):
    CK = 128
    NQ = S // TQ
    NC = S // CK
    NSTEP = H * NQ
    NX = S // TP1
    NO = S // TM
    assert UN % 2 == 0 and (NSTEP - 2) % UN == 0

    def kernel(x_hbm, wqkv_hbm, wo_hbm, wg_hbm, wu_hbm, wd_hbm, o_hbm,
               x_v, wqkv_v, wo_v, wg_v, wu_v, wd_v, o_v,
               k_s, qt_s, vt_s, ot_s, s0, s1, w0, w1, sem_x, sem_w, sem_o):
        s_bufs = (s0, s1)
        w_bufs = (w0, w1)

        def x_copy(j):
            r = pl.ds(j * TP1, TP1)
            return pltpu.make_async_copy(x_hbm.at[r], x_v.at[r], sem_x.at[j])

        def o_copy(j):
            r = pl.ds(j * TM, TM)
            return pltpu.make_async_copy(o_v.at[r], o_hbm.at[r], sem_o.at[j])

        w_copies = [pltpu.make_async_copy(a, b, sem_w.at[i]) for i, (a, b) in enumerate(
            [(wqkv_hbm, wqkv_v), (wo_hbm, wo_v), (wg_hbm, wg_v), (wu_hbm, wu_v), (wd_hbm, wd_v)])]

        x_copy(0).start()
        w_copies[0].start()
        for j in range(1, NX):
            x_copy(j).start()

        x_copy(0).wait()
        xn0 = _ln(x_v[0:TP1, :].astype(F32)).astype(BF16)
        w_copies[0].wait()
        for j in range(1, NX):
            x_copy(j).wait()
        for cp in w_copies[1:]:
            cp.start()
        wqT = wqkv_v[:, 0:D].astype(F32).T.astype(BF16)
        wvT = wqkv_v[:, 2 * D:3 * D].astype(F32).T.astype(BF16)
        wk = wqkv_v[:, D:2 * D]
        nt = (((1,), (1,)), ((), ()))
        for j in range(NX if P1 else 0):
            rows = slice(j * TP1, (j + 1) * TP1)
            hrows = slice(j * TP1 // 2, (j + 1) * TP1 // 2)
            xn = xn0 if j == 0 else _ln(x_v[rows, :].astype(F32)).astype(BF16)
            kk = _pk(jnp.dot(xn, wk, preferred_element_type=F32).astype(BF16))
            for g in range(4):
                k_s[g, hrows, :] = kk[:, g * 128:(g + 1) * 128]
            qt = lax.dot_general(wqT, xn, nt, preferred_element_type=F32)
            jq, off = (j * TP1) // TQ, (j * TP1) % TQ
            qt_s[jq, :, off:off + TP1] = _pk((qt * QSCALE).astype(BF16))
            vt = lax.dot_general(wvT, xn, nt, preferred_element_type=F32)
            vt_s[:, rows] = _pk(vt.astype(BF16))

        def set_w(w_s, t):
            j = t // H
            h = t % H
            w_s[...] = jnp.zeros((64, TQ), U32)
            src = pl.multiple_of(h * 8, 8)
            dst = pl.multiple_of((h % 8) * 8, 8)
            w_s[pl.ds(dst, 8), :] = qt_s[j, pl.ds(src, 8), :]

        def a_chunk(t, par, c, m8):
            g = (t % H) // 8
            s = jnp.dot(_up(k_s[g, c * 64:(c + 1) * 64, :]), _up(w_bufs[par][...]),
                        preferred_element_type=F32)
            s_bufs[par][c * CK:(c + 1) * CK, :] = s
            cm = jnp.max(s.reshape(16, 8, TQ), axis=0)
            return (cm if m8 is None else jnp.maximum(m8, cm)), s[0:8, :]

        def b_chunk(t, par, c, st, m_c):
            acc, l8, m_b = st
            hrow = pl.multiple_of((t % H) * 8, 8)
            ks = slice(c * CK, (c + 1) * CK)
            p = jnp.exp2(s_bufs[par][ks, :].reshape(16, 8, TQ) - m_c[None]).reshape(CK, TQ)
            for i in reversed(range(8)):
                l8 = l8 + (p[16 * i:16 * i + 8, :] + p[16 * i + 8:16 * i + 16, :])
            acc = acc + jnp.dot(_up(vt_s[pl.ds(hrow, 8), ks]), p.astype(BF16),
                                preferred_element_type=F32)
            return acc, l8, m_b

        def b_fin(t, st):
            acc, l8, _ = st
            hrow = pl.multiple_of((t % H) * 8, 8)
            l = jnp.sum(l8, axis=0, keepdims=True)
            ot_s[t // H, pl.ds(hrow, 8), :] = _pk((acc / l).astype(BF16))

        def b_init(m8):
            m_b = jnp.broadcast_to(jnp.max(m8, axis=0, keepdims=True), (8, TQ))
            return jnp.zeros((DH, TQ), F32), jnp.zeros((8, TQ), F32), m_b

        def run_slots(slots, st, m8_prev, never):
            deps = []
            for (s, par, do_a, pre_w) in slots:
                if pre_w:
                    set_w(w_bufs[1 - par], s + 1)
                m8 = None
                for c in range(NC):
                    if do_a:
                        m8, dep = a_chunk(s, par, c, m8)
                        deps.append(dep)
                    else:
                        deps.append(None)
                    if c == DELAY:
                        st = b_init(m8_prev)
                    dep = deps[-1 - FENCE] if len(deps) > FENCE else None
                    m_c = st[2] if dep is None else jnp.where(never, dep, st[2])
                    if c < DELAY:
                        tb = jnp.maximum(s - 2, 0)
                        st = b_chunk(tb, par, NC - DELAY + c, st, m_c)
                        if c == DELAY - 1:
                            b_fin(tb, st)
                    else:
                        st = b_chunk(s - 1, 1 - par, c - DELAY, st, m_c)
                m8_prev = m8
            return st, m8_prev

        if P2:
            set_w(w_bufs[0], 0)
            set_w(w_bufs[1], 1)
            s1[(NC - DELAY) * CK:, :] = jnp.zeros((DELAY * CK, TQ), F32)
            m8 = None
            for c in range(NC):
                m8, _ = a_chunk(0, 0, c, m8)
            st = (jnp.zeros((DH, TQ), F32), jnp.ones((8, TQ), F32), jnp.zeros((8, TQ), F32))

            def body(i, carry):
                st, m8, _ = carry
                s_base = 1 + UN * i
                slots = [(s_base + u, (1 + u) % 2, True, True) for u in range(UN)]
                st, m8 = run_slots(slots, st, m8, i < 0)
                return st, m8, i

            st, m8, last = lax.fori_loop(0, (NSTEP - 2) // UN, body, (st, m8, jnp.int32(0)))
            st, _ = run_slots([(NSTEP - 1, 1, True, False), (NSTEP, 0, False, False)],
                              st, m8, last < 0)
            for c in range(NC - DELAY, NC):
                st = b_chunk(NSTEP - 1, 1, c, st, st[2])
            b_fin(NSTEP - 1, st)

        for cp in w_copies[1:]:
            cp.wait()
        tn = (((0,), (0,)), ((), ()))
        for j in range(NO):
            rows = slice(j * TM, (j + 1) * TM)
            if P3:
                jq, off = (j * TM) // TQ, (j * TM) % TQ
                attn = lax.dot_general(_up(ot_s[jq, :, off:off + TM]), wo_v[...], tn,
                                       preferred_element_type=F32)
                h = x_v[rows, :].astype(F32) + attn
                hn = _ln(h).astype(BF16)
                gt = lax.dot_general(hn, wg_v[...], nt, preferred_element_type=F32)
                up = lax.dot_general(hn, wu_v[...], nt, preferred_element_type=F32)
                a = (_gelu_tanh(gt) * up).astype(BF16)
                y = jnp.dot(a, wd_v[...], preferred_element_type=F32)
                o_v[rows, :] = (h + y).astype(BF16)
            else:
                o_v[rows, :] = x_v[rows, :]
            o_copy(j).start()
        for j in range(NO):
            o_copy(j).wait()

    @jax.jit
    def fn(A_x, A_wqkv, A_wo, B_x, B_w_gate, B_w_up, B_w_down):
        x = A_x.reshape(S, D)
        anyspec = pl.BlockSpec(memory_space=pltpu.MemorySpace.HBM)
        out = pl.pallas_call(
            kernel,
            out_shape=jax.ShapeDtypeStruct((S, D), BF16),
            in_specs=[anyspec] * 6,
            out_specs=anyspec,
            scratch_shapes=[
                pltpu.VMEM((S, D), BF16),
                pltpu.VMEM((D, 3 * D), BF16),
                pltpu.VMEM((D, D), BF16),
                pltpu.VMEM((F, D), BF16),
                pltpu.VMEM((F, D), BF16),
                pltpu.VMEM((F, D), BF16),
                pltpu.VMEM((S, D), BF16),
                pltpu.VMEM((4, S // 2, 128), U32),
                pltpu.VMEM((NQ, D // 2, TQ), U32),
                pltpu.VMEM((D // 2, S), U32),
                pltpu.VMEM((NQ, D // 2, TQ), U32),
                pltpu.VMEM((S, TQ), F32),
                pltpu.VMEM((S, TQ), F32),
                pltpu.VMEM((64, TQ), U32),
                pltpu.VMEM((64, TQ), U32),
                pltpu.SemaphoreType.DMA((NX,)),
                pltpu.SemaphoreType.DMA((5,)),
                pltpu.SemaphoreType.DMA((NO,)),
            ],
            compiler_params=pltpu.CompilerParams(vmem_limit_bytes=100 * 2 ** 20),
        )(x, A_wqkv, A_wo, B_w_gate.T, B_w_up.T, B_w_down)
        return out.reshape(1, S, D)

    return fn


_impl = make()


@jax.jit
def pallas_sequential_preLN__softmax_full_mha__geglu_ffn__prompt_kernel(A_x, A_wqkv, A_wo, B_x, B_w_gate, B_w_up, B_w_down):
    return _impl(A_x, A_wqkv, A_wo, B_x, B_w_gate, B_w_up, B_w_down)
```

```python
import math

import jax
import jax.numpy as jnp
from jax import lax
import jax.experimental.pallas as pl
import jax.experimental.pallas.tpu as pltpu

S, D, H, DH, F = 2048, 512, 32, 16, 1376
EPS = 1e-5
QSCALE = (DH ** -0.5) * math.log2(math.e)
F32, BF16, U32 = jnp.float32, jnp.bfloat16, jnp.uint32
L_MIN, L_MAX, ACC_MAX = 2.0 ** -20, 2.0 ** 100, 2.0 ** 120

TQ = 512
CK = 128
KV = 256
PSZ = 32
NQ, NL, NC = S // TQ, TQ // 128, S // CK
HPB = 2
UN = HPB * NQ
CA = (S - KV) // NC
NPK = KV // PSZ
NP = NPK * NL
KB_END = 60
B_ORDER = [2, 3, 4, 5, 0, 1] + list(range(6, NC))
XT = (256, 256, 512, 512, 512)
OT = (512, 512, 512, 256, 256)
XS = [sum(XT[:i]) for i in range(len(XT))]
OS = [sum(OT[:i]) for i in range(len(OT))]
FM = (F // 128) * 128
NT = (((1,), (1,)), ((), ()))
TN = (((0,), (0,)), ((), ()))

KB_AT = [[q for q in range(4 * DH) if (q * KB_END) // (4 * DH) == p] for p in range(NQ * NC)]
_N16 = (S - KV) // 16
KR_AT = [(min(_N16, (p * _N16) // KB_END), min(_N16, ((p + 1) * _N16) // KB_END))
         for p in range(NQ * NC)]


def _block_slots(c0):
    nh = 2 * (NC - c0)
    return {(c0 + t // 2, t % 2): [k for k in range(NP) if (k * nh) // NP == t]
            for t in range(nh)}


def _ln(x):
    m = jnp.mean(x, axis=-1, keepdims=True)
    xc = x - m
    v = jnp.mean(xc * xc, axis=-1, keepdims=True)
    return xc * lax.rsqrt(v + EPS)


def _gelu_tanh(x):
    c = math.sqrt(2.0 / math.pi)
    return 0.5 * x * (1.0 + jnp.tanh(c * (x + 0.044715 * (x * x * x))))


def _pk(x):
    return pltpu.bitcast(x, U32)


def _up(x):
    return pltpu.bitcast(x, BF16)


def _al(x):
    return pl.multiple_of(x, 8)


def _kernel(x_hbm, wqkv_hbm, wo_hbm, wg_hbm, wu_hbm, wd_hbm, o_hbm,
            x_v, wqkv_v, wo_v, wg_v, wu_v, wd_v, o_v,
            k_s, qt_s, vt_s, ot_s, p0, p1, pv0, pv1, w_s, kr0, kr1, kb0, kb1,
            s_s, h_s, hn_s, sem_x, sem_w, sem_o):
    p_bufs, pv_bufs = (p0, p1), (pv0, pv1)
    kr_bufs, kb_bufs = (kr0, kr1), (kb0, kb1)

    def x_copy(j):
        r = pl.ds(XS[j], XT[j])
        return pltpu.make_async_copy(x_hbm.at[r], x_v.at[r], sem_x.at[j])

    def o_copy(j):
        r = pl.ds(OS[j], OT[j])
        return pltpu.make_async_copy(o_v.at[r], o_hbm.at[r], sem_o.at[j])

    def qkv_copy(p):
        return pltpu.make_async_copy(wqkv_hbm.at[:, pl.ds(p * D, D)], wqkv_v.at[p], sem_w.at[p])

    w_copies = [pltpu.make_async_copy(a, b, sem_w.at[3 + i]) for i, (a, b) in enumerate(
        [(wo_hbm, wo_v), (wg_hbm, wg_v), (wu_hbm, wu_v), (wd_hbm, wd_v)])]

    x_copy(0).start()
    qkv_copy(1).start()
    p1[...] = jnp.zeros(p1.shape, U32)
    pv1[...] = jnp.zeros(pv1.shape, U32)

    def ln_x(j):
        return _ln(x_v[XS[j]:XS[j] + XT[j], :].astype(F32)).astype(BF16)

    def proj_k(j, xn, g0=0, g1=4):
        r0, n = XS[j], XT[j]
        kk = _pk(jnp.dot(xn, wqkv_v[1, :, g0 * 128:g1 * 128],
                         preferred_element_type=F32).astype(BF16))
        for g in range(g0, g1):
            k_s[g, r0 // 2:(r0 + n) // 2, :] = kk[:, (g - g0) * 128:(g - g0 + 1) * 128]

    def proj_qv(j, xn, wq_t, wv_t):
        r0, n = XS[j], XT[j]
        qt = lax.dot_general(wq_t, xn, NT, preferred_element_type=F32)
        qt_s[r0 // TQ, :, r0 % TQ:r0 % TQ + n] = _pk((qt * QSCALE).astype(BF16))
        vt = lax.dot_general(wv_t, xn, NT, preferred_element_type=F32)
        vt_s[:, r0:r0 + n] = _pk(vt.astype(BF16))

    x_copy(0).wait()
    x_copy(1).start()
    xns = [ln_x(0)]
    qkv_copy(1).wait()
    x_copy(2).start()
    x_copy(3).start()
    x_copy(1).wait()
    x_copy(4).start()
    proj_k(0, xns[0])
    xns.append(ln_x(1))
    proj_k(1, xns[1], 0, 2)
    x_copy(2).wait()
    proj_k(1, xns[1], 2, 4)
    xns.append(ln_x(2))
    proj_k(2, xns[2], 0, 2)
    x_copy(3).wait()
    x_copy(4).wait()
    qkv_copy(0).start()
    qkv_copy(2).start()
    proj_k(2, xns[2], 2, 4)
    xns.append(ln_x(3))
    proj_k(3, xns[3])
    xns.append(ln_x(4))
    proj_k(4, xns[4], 0, 2)
    qkv_copy(0).wait()
    qkv_copy(2).wait()
    for cp in w_copies:
        cp.start()
    proj_k(4, xns[4], 2, 4)
    wq_t = wqkv_v[0].astype(F32).T.astype(BF16)
    wv_t = wqkv_v[2].astype(F32).T.astype(BF16)

    def set_kr(hp, h, v0, v1):
        kp = k_s[h // 8, KV // 2 + 8 * v0:KV // 2 + 8 * v1, :]
        kr_bufs[hp][8 * v0:8 * v1, :] = pltpu.roll(kp, (128 - (h % 8) * DH) % 128, 1)

    def set_kb(hp, h, d, r0, r1, never=None, dep=None):
        n = r1 - r0
        kp = k_s[h // 8, r0 // 2:r1 // 2, :]
        if dep is not None:
            kp = jnp.where(never, _pk(dep[0:n // 2, 0:128]), kp)
        idx = jnp.full((n // 2, 128), (h % 8) * DH + d, jnp.int32)
        kb_bufs[hp][d * KV + r0:d * KV + r1, :] = _up(
            jnp.take_along_axis(kp, idx, axis=1)).astype(F32)

    for d in range(DH):
        set_kb(0, 0, d, 0, KV)
    kr0[...] = k_s[0, KV // 2:, :]
    for j in range(len(XT)):
        proj_qv(j, xns[j], wq_t, wv_t)

    def hook(w, never, deps, row, t0):
        if not deps:
            return w
        tiles = [w[row:row + 8, n * 128:(n + 1) * 128] for n in range(NL)]
        for t, dep in enumerate(deps):
            t = (t + t0) % NL
            tiles[t] = jnp.where(never, _pk(dep), tiles[t])
        rows = [w[0:row, :]] if row else []
        return jnp.concatenate(rows + [jnp.concatenate(tiles, axis=1)], axis=0)

    def a_chunk(h, j, hp, par, c, l8, never, deps):
        r0 = c * CA
        kp = kr_bufs[hp][r0 // 2:(r0 + CA) // 2, :]
        w = hook(qt_s[j, pl.ds(_al(h * 8), 8), :], never, deps, 0, 3)
        s = jnp.dot(_up(kp)[:, 0:DH], _up(w), preferred_element_type=F32)
        p = jnp.exp2(s)
        p_bufs[par][r0 // 2:(r0 + CA) // 2, :] = _pk(p.astype(BF16))
        for i in range(CA // 16):
            t = p[16 * i:16 * i + 8, :] + p[16 * i + 8:16 * i + 16, :]
            l8 = t if l8 is None else l8 + t
        return l8, s

    def v_block(h, j, hp, par, k, lv, never, zero, dep):
        n, r0 = k // NPK, (k % NPK) * PSZ
        qp = qt_s[j, pl.ds(_al(h * 8), 8), n * 128:(n + 1) * 128]
        if dep is not None:
            qp = jnp.where(never, _pk(dep), qp)
        qf = _up(qp).astype(F32)
        acc = None
        for d in range(DH):
            t = kb_bufs[hp][pl.ds(_al(d * KV + r0 + zero * 8), PSZ), :] * qf[d:d + 1, :]
            acc = t if acc is None else acc + t
        p = jnp.exp2(acc)
        t = (p[0:8] + p[8:16]) + (p[16:24] + p[24:32])
        lv[n] = t if lv[n] is None else lv[n] + t
        pv_bufs[par][r0 // 2:(r0 + PSZ) // 2, n * 128:(n + 1) * 128] = _pk(p.astype(BF16))
        return lv[n]

    def b_chunk(h, par, c, acc, zero, never=None, dep=None, deps=()):
        vt = vt_s[pl.ds(_al(h * 8), 8), c * CK:(c + 1) * CK]
        if dep is not None:
            vt = jnp.where(never, _pk(dep), vt)
        if c * CK < KV:
            pt = pv_bufs[par][pl.ds(_al(c * CK // 2 + zero * 8), CK // 2), :]
        else:
            pt = p_bufs[par][(c * CK - KV) // 2:((c + 1) * CK - KV) // 2, :]
        pt = hook(pt, never, deps, CK // 2 - 8, 0)
        return acc + jnp.dot(_up(vt), _up(pt), preferred_element_type=F32)

    def b_fin(h, j, acc, l8, ok):
        l = jnp.sum(l8, axis=0, keepdims=True)
        ot_s[j, pl.ds(_al(h * 8), 8), :] = _pk((acc / l).astype(BF16))
        amax = jnp.maximum(jnp.abs(acc[0:8]), jnp.abs(acc[8:16]))
        good = (amax <= ACC_MAX) & (l >= L_MIN) & (l <= L_MAX)
        return jnp.where(good, ok, 0.0)

    def body(i, carry):
        l_prev, acc, ok = carry
        never = i < 0
        zero = lax.shift_right_logical(i, 16)
        scores = []
        due = {}
        for u in range(UN):
            par, hp, j = u % 2, (u // NQ) % 2, u % NQ
            h = HPB * i + u // NQ
            h_b = jnp.maximum(HPB * i + (u - 1) // NQ, 0)
            h_k = jnp.minimum(h + 1, H - 1)
            lv = [None] * NL
            l8 = None
            acc = jnp.where(never, acc, 0.0)
            blocks = _block_slots(1 if u == 0 else 0)
            for c in range(NC):
                pos = u * NC + c
                rel = scores[-2][0:8, 0:128] if len(scores) >= 2 else None
                hk = [[v_block(h, j, hp, par, k, lv, never,
                               lax.shift_right_logical(i + (u * NL + k // NPK), 16), rel)
                       for k in blocks.get((c, t), [])] for t in range(2)]
                l8, s = a_chunk(h, j, hp, par, c, l8, never, hk[0])
                prev = scores[-1] if scores else None
                scores.append(s)
                for q in KB_AT[j * NC + c]:
                    set_kb(1 - hp, h_k, q // 4, (q % 4) * (KV // 4), (q % 4 + 1) * (KV // 4),
                           never, prev)
                v0, v1 = KR_AT[j * NC + c]
                if v1 > v0:
                    set_kr(1 - hp, h_k, v0, v1)
                    kq = kr_bufs[1 - hp][pl.ds(_al(zero * 8), 8), :]
                    due.setdefault(pos + 1, []).append(pltpu.bitcast(kq, F32))
                dep = None
                for e in due.get(pos, []):
                    dep = e if dep is None else dep + e
                if KB_AT[j * NC + c]:
                    due.setdefault(pos + 1, []).insert(
                        0, kb_bufs[1 - hp][pl.ds(_al(zero * 8), 8), :])
                pp = p_bufs[par][pl.ds(_al(zero * 8), 8), 0:128]
                n0 = (c % NL) * 128
                due.setdefault(pos + 2, []).extend([pltpu.bitcast(pp, F32), l8[:, n0:n0 + 128]])
                acc = b_chunk(h_b, 1 - par, B_ORDER[c], acc, zero, never, dep, hk[1])
            ok = b_fin(h_b, (u - 1) % NQ, acc, l_prev, ok)
            l_prev = l8 + jnp.concatenate(lv, axis=1)
        return l_prev, acc, ok

    for cp in w_copies:
        cp.wait()
    ones = jnp.ones((8, TQ), F32)
    l_prev, _, ok = lax.fori_loop(0, H // HPB, body, (ones, jnp.zeros((DH, TQ), F32), ones))

    def pre(j, ln=True):
        r0, n = OS[j], OT[j]
        attn = lax.dot_general(_up(ot_s[r0 // TQ, :, r0 % TQ:r0 % TQ + n]), wo_v[...], TN,
                               preferred_element_type=F32)
        h = x_v[r0:r0 + n, :].astype(F32) + attn
        h_s[r0:r0 + n, :] = h
        if ln:
            hn_s[r0 // 2:(r0 + n) // 2, :] = _pk(_ln(h).astype(BF16))

    acc = jnp.zeros((DH, TQ), F32)
    for c in range(NC):
        acc = b_chunk(H - 1, 1, B_ORDER[c], acc, 0)
    ok = b_fin(H - 1, NQ - 1, acc, l_prev, ok)
    pre(0)
    pre(1, ln=False)

    @pl.when(jnp.min(ok) < 0.5)
    def _attention_with_row_max():
        def step(t, carry):
            h, j = t // NQ, t % NQ
            hrow = _al(h * 8)
            w_s[...] = jnp.zeros(w_s.shape, U32)
            w_s[pl.ds(_al((h % 8) * 8), 8), :] = qt_s[j, pl.ds(hrow, 8), :]
            s_s[...] = jnp.dot(_up(k_s[h // 8]), _up(w_s[...]), preferred_element_type=F32)
            m = jnp.max(s_s[...], axis=0, keepdims=True)
            p = jnp.exp2(s_s[...] - m)
            l = jnp.sum(p, axis=0, keepdims=True)
            o = jnp.dot(_up(vt_s[pl.ds(hrow, 8), :]), p.astype(BF16),
                        preferred_element_type=F32)
            ot_s[j, pl.ds(hrow, 8), :] = _pk((o / l).astype(BF16))
            return carry

        lax.fori_loop(0, H * NQ, step, 0)
        pre(0)
        pre(1, ln=False)

    def ffn(j):
        r0, n = OS[j], OT[j]
        hn = _up(hn_s[r0 // 2:(r0 + n) // 2, :])
        w_rem = jnp.concatenate([wg_v[FM:F, :], wu_v[FM:F, :]], axis=0)
        rem_t = lax.dot_general(w_rem, hn, NT, preferred_element_type=F32)
        a_rem_t = (_gelu_tanh(rem_t[0:F - FM]) * rem_t[F - FM:]).astype(BF16)
        gate = lax.dot_general(hn, wg_v[0:FM, :], NT, preferred_element_type=F32)
        up = lax.dot_general(hn, wu_v[0:FM, :], NT, preferred_element_type=F32)
        a = (_gelu_tanh(gate) * up).astype(BF16)
        y = (jnp.dot(a, wd_v[0:FM, :], preferred_element_type=F32)
             + lax.dot_general(a_rem_t, wd_v[FM:F, :], TN, preferred_element_type=F32))
        o_v[r0:r0 + n, :] = (h_s[r0:r0 + n, :] + y).astype(BF16)

    hn_s[OS[1] // 2:OS[2] // 2, :] = _pk(_ln(h_s[OS[1]:OS[2], :]).astype(BF16))
    for j in range(len(OT)):
        if j + 2 < len(OT):
            pre(j + 2)
        ffn(j)
        o_copy(j).start()
    for j in range(len(OT)):
        o_copy(j).wait()


def _call(x, wqkv, wo, wg_t, wu_t, wd, interpret=False):
    hbm = pl.BlockSpec(memory_space=pltpu.MemorySpace.HBM)
    return pl.pallas_call(
        _kernel,
        out_shape=jax.ShapeDtypeStruct((S, D), BF16),
        in_specs=[hbm] * 6,
        out_specs=hbm,
        scratch_shapes=[
            pltpu.VMEM((S, D), BF16),
            pltpu.VMEM((3, D, D), BF16),
            pltpu.VMEM((D, D), BF16),
            pltpu.VMEM((F, D), BF16),
            pltpu.VMEM((F, D), BF16),
            pltpu.VMEM((F, D), BF16),
            pltpu.VMEM((S, D), BF16),
            pltpu.VMEM((4, S // 2, 128), U32),
            pltpu.VMEM((NQ, D // 2, TQ), U32),
            pltpu.VMEM((D // 2, S), U32),
            pltpu.VMEM((NQ, D // 2, TQ), U32),
            pltpu.VMEM(((S - KV) // 2, TQ), U32),
            pltpu.VMEM(((S - KV) // 2, TQ), U32),
            pltpu.VMEM((KV // 2, TQ), U32),
            pltpu.VMEM((KV // 2, TQ), U32),
            pltpu.VMEM((64, TQ), U32),
            pltpu.VMEM(((S - KV) // 2, 128), U32),
            pltpu.VMEM(((S - KV) // 2, 128), U32),
            pltpu.VMEM((DH * KV, 128), F32),
            pltpu.VMEM((DH * KV, 128), F32),
            pltpu.VMEM((S, TQ), F32),
            pltpu.VMEM((S, D), F32),
            pltpu.VMEM((S // 2, D), U32),
            pltpu.SemaphoreType.DMA((len(XT),)),
            pltpu.SemaphoreType.DMA((7,)),
            pltpu.SemaphoreType.DMA((len(OT),)),
        ],
        compiler_params=pltpu.CompilerParams(vmem_limit_bytes=100 * 2 ** 20),
        interpret=interpret,
    )(x, wqkv, wo, wg_t, wu_t, wd)


@jax.jit
def pallas_sequential_preLN__softmax_full_mha__geglu_ffn__prompt_kernel(
    A_x: jax.Array,
    A_wqkv: jax.Array,
    A_wo: jax.Array,
    B_x: jax.Array,
    B_w_gate: jax.Array,
    B_w_up: jax.Array,
    B_w_down: jax.Array,
):
    out = _call(A_x.reshape(S, D), A_wqkv, A_wo, B_w_gate.T, B_w_up.T, B_w_down)
    return out.reshape(1, S, D)
```

```python
import math

import jax
import jax.numpy as jnp
from jax import lax
import jax.experimental.pallas as pl
import jax.experimental.pallas.tpu as pltpu

S, D, H, DH, F = 2048, 512, 32, 16, 1376
EPS = 1e-5
QSCALE = (DH ** -0.5) * math.log2(math.e)
F32, BF16, U32 = jnp.float32, jnp.bfloat16, jnp.uint32
L_MIN, L_MAX, ACC_MAX = 2.0 ** -20, 2.0 ** 100, 2.0 ** 120

TQ = 512
CK = 128
KV = 256
PSZ = 32
NQ, NL, NC = S // TQ, TQ // 128, S // CK
HPB = 2
UN = HPB * NQ
CA = (S - KV) // NC
NPK = KV // PSZ
NP = NPK * NL
KB_END = 60
B_ORDER = [2, 3, 4, 5, 0, 1] + list(range(6, NC))
XT = (256, 256, 512, 512, 512)
OT = (512, 512, 512, 256, 128, 128)
XS = [sum(XT[:i]) for i in range(len(XT))]
OS = [sum(OT[:i]) for i in range(len(OT))]
FM = (F // 128) * 128
NT = (((1,), (1,)), ((), ()))
TN = (((0,), (0,)), ((), ()))

KB_AT = [[q for q in range(4 * DH) if (q * KB_END) // (4 * DH) == p] for p in range(NQ * NC)]
_N16 = (S - KV) // 16
KR_AT = [(min(_N16, (p * _N16) // KB_END), min(_N16, ((p + 1) * _N16) // KB_END))
         for p in range(NQ * NC)]


def _block_slots(c0):
    nh = 2 * (NC - c0)
    return {(c0 + t // 2, t % 2): [k for k in range(NP) if (k * nh) // NP == t]
            for t in range(nh)}


def _ln(x):
    m = jnp.mean(x, axis=-1, keepdims=True)
    xc = x - m
    v = jnp.mean(xc * xc, axis=-1, keepdims=True)
    return xc * lax.rsqrt(v + EPS)


def _gelu_tanh(x):
    c = math.sqrt(2.0 / math.pi)
    return 0.5 * x * (1.0 + jnp.tanh(c * (x + 0.044715 * (x * x * x))))


def _pk(x):
    return pltpu.bitcast(x, U32)


def _up(x):
    return pltpu.bitcast(x, BF16)


def _al(x):
    return pl.multiple_of(x, 8)


def _kernel(x_hbm, wqkv_hbm, wo_hbm, wg_hbm, wu_hbm, wd_hbm, o_hbm,
            x_v, wqkv_v, wo_v, wg_v, wu_v, wd_v, o_v,
            k_s, qt_s, vt_s, ot_s, p0, p1, pv0, pv1, w_s, kr0, kr1, kb0, kb1,
            s_s, h_s, hn_s, sem_x, sem_w, sem_o):
    p_bufs, pv_bufs = (p0, p1), (pv0, pv1)
    kr_bufs, kb_bufs = (kr0, kr1), (kb0, kb1)

    def x_copy(j):
        r = pl.ds(XS[j], XT[j])
        return pltpu.make_async_copy(x_hbm.at[r], x_v.at[r], sem_x.at[j])

    def o_copy(j):
        r = pl.ds(OS[j], OT[j])
        return pltpu.make_async_copy(o_v.at[r], o_hbm.at[r], sem_o.at[j])

    def qkv_copy(p):
        return pltpu.make_async_copy(wqkv_hbm.at[:, pl.ds(p * D, D)], wqkv_v.at[p], sem_w.at[p])

    w_copies = [pltpu.make_async_copy(a, b, sem_w.at[3 + i]) for i, (a, b) in enumerate(
        [(wo_hbm, wo_v), (wg_hbm, wg_v), (wu_hbm, wu_v), (wd_hbm, wd_v)])]

    x_copy(0).start()
    qkv_copy(1).start()
    p1[...] = jnp.zeros(p1.shape, U32)
    pv1[...] = jnp.zeros(pv1.shape, U32)

    def ln_x(j):
        return _ln(x_v[XS[j]:XS[j] + XT[j], :].astype(F32)).astype(BF16)

    def proj_k(j, xn, g0=0, g1=4):
        r0, n = XS[j], XT[j]
        kk = _pk(jnp.dot(xn, wqkv_v[1, :, g0 * 128:g1 * 128],
                         preferred_element_type=F32).astype(BF16))
        for g in range(g0, g1):
            k_s[g, r0 // 2:(r0 + n) // 2, :] = kk[:, (g - g0) * 128:(g - g0 + 1) * 128]

    def proj_qv(j, xn, wq_t, wv_t):
        r0, n = XS[j], XT[j]
        qt = lax.dot_general(wq_t, xn, NT, preferred_element_type=F32)
        qt_s[r0 // TQ, :, r0 % TQ:r0 % TQ + n] = _pk((qt * QSCALE).astype(BF16))
        vt = lax.dot_general(wv_t, xn, NT, preferred_element_type=F32)
        vt_s[:, r0:r0 + n] = _pk(vt.astype(BF16))

    x_copy(0).wait()
    x_copy(1).start()
    xns = [ln_x(0)]
    qkv_copy(1).wait()
    x_copy(2).start()
    x_copy(3).start()
    x_copy(1).wait()
    x_copy(4).start()
    proj_k(0, xns[0])
    xns.append(ln_x(1))
    proj_k(1, xns[1], 0, 2)
    x_copy(2).wait()
    proj_k(1, xns[1], 2, 4)
    xns.append(ln_x(2))
    proj_k(2, xns[2], 0, 2)
    x_copy(3).wait()
    x_copy(4).wait()
    qkv_copy(0).start()
    qkv_copy(2).start()
    proj_k(2, xns[2], 2, 4)
    xns.append(ln_x(3))
    proj_k(3, xns[3])
    xns.append(ln_x(4))
    proj_k(4, xns[4], 0, 2)
    qkv_copy(0).wait()
    qkv_copy(2).wait()
    for cp in w_copies:
        cp.start()
    proj_k(4, xns[4], 2, 4)
    wq_t = wqkv_v[0].astype(F32).T.astype(BF16)
    wv_t = wqkv_v[2].astype(F32).T.astype(BF16)

    def set_kr(hp, h, v0, v1):
        kp = k_s[h // 8, KV // 2 + 8 * v0:KV // 2 + 8 * v1, :]
        kr_bufs[hp][8 * v0:8 * v1, :] = pltpu.roll(kp, (128 - (h % 8) * DH) % 128, 1)

    def set_kb(hp, h, d, r0, r1, never=None, dep=None):
        n = r1 - r0
        kp = k_s[h // 8, r0 // 2:r1 // 2, :]
        if dep is not None:
            kp = jnp.where(never, _pk(dep[0:n // 2, 0:128]), kp)
        idx = jnp.full((n // 2, 128), (h % 8) * DH + d, jnp.int32)
        kb_bufs[hp][d * KV + r0:d * KV + r1, :] = _up(
            jnp.take_along_axis(kp, idx, axis=1)).astype(F32)

    for d in range(DH):
        set_kb(0, 0, d, 0, KV)
    kr0[...] = k_s[0, KV // 2:, :]
    for j in range(len(XT)):
        proj_qv(j, xns[j], wq_t, wv_t)

    def hook(w, never, deps):
        if not deps:
            return w
        row = w.shape[0] - 8
        tiles = [w[row:row + 8, n * 128:(n + 1) * 128] for n in range(NL)]
        for t, dep in enumerate(deps):
            tiles[t] = jnp.where(never, _pk(dep), tiles[t])
        rows = [w[0:row, :]] if row else []
        return jnp.concatenate(rows + [jnp.concatenate(tiles, axis=1)], axis=0)

    def a_chunk(h, j, hp, par, c, l8, never, deps):
        r0 = c * CA
        kp = kr_bufs[hp][r0 // 2:(r0 + CA) // 2, :]
        w = hook(qt_s[j, pl.ds(_al(h * 8), 8), :], never, deps)
        s = jnp.dot(_up(kp)[:, 0:DH], _up(w), preferred_element_type=F32)
        p = jnp.exp2(s)
        p_bufs[par][r0 // 2:(r0 + CA) // 2, :] = _pk(p.astype(BF16))
        for i in range(CA // 16):
            t = p[16 * i:16 * i + 8, :] + p[16 * i + 8:16 * i + 16, :]
            l8 = t if l8 is None else l8 + t
        return l8, s

    def v_block(h, j, hp, par, k, lv, never, zero, dep):
        n, r0 = k // NPK, (k % NPK) * PSZ
        qp = qt_s[j, pl.ds(_al(h * 8), 8), n * 128:(n + 1) * 128]
        if dep is not None:
            qp = jnp.where(never, _pk(dep), qp)
        qf = _up(qp).astype(F32)
        acc = None
        for d in range(DH):
            t = kb_bufs[hp][pl.ds(_al(d * KV + r0 + zero * 8), PSZ), :] * qf[d:d + 1, :]
            acc = t if acc is None else acc + t
        p = jnp.exp2(acc)
        t = (p[0:8] + p[8:16]) + (p[16:24] + p[24:32])
        lv[n] = t if lv[n] is None else lv[n] + t
        pv_bufs[par][r0 // 2:(r0 + PSZ) // 2, n * 128:(n + 1) * 128] = _pk(p.astype(BF16))
        return lv[n]

    def b_chunk(h, par, c, acc, zero, never=None, deps=()):
        vt = vt_s[pl.ds(_al(h * 8), 8), c * CK:(c + 1) * CK]
        if c * CK < KV:
            pt = pv_bufs[par][pl.ds(_al(c * CK // 2 + zero * 8), CK // 2), :]
        else:
            pt = p_bufs[par][(c * CK - KV) // 2:((c + 1) * CK - KV) // 2, :]
        pt = hook(pt, never, deps)
        return acc + jnp.dot(_up(vt), _up(pt), preferred_element_type=F32)

    def b_fin(h, j, acc, l8, ok):
        l = jnp.sum(l8, axis=0, keepdims=True)
        r = pl.reciprocal(l, approx=True)
        r = r * (2.0 - l * r)
        ot_s[j, pl.ds(_al(h * 8), 8), :] = _pk((acc * r).astype(BF16))
        good = ((jnp.abs(acc[0:8]) <= ACC_MAX) & (jnp.abs(acc[8:16]) <= ACC_MAX)
                & (l >= L_MIN) & (l <= L_MAX))
        return jnp.where(good, ok, 0.0)

    def body(i, carry):
        l_prev, acc, ok = carry
        never = i < 0
        zero = lax.shift_right_logical(i, 16)
        scores = []
        due = {}
        for u in range(UN):
            par, hp, j = u % 2, (u // NQ) % 2, u % NQ
            h = HPB * i + u // NQ
            h_b = jnp.maximum(HPB * i + (u - 1) // NQ, 0)
            h_k = jnp.minimum(h + 1, H - 1)
            lv = [None] * NL
            l8 = None
            acc = jnp.where(never, acc, 0.0)
            blocks = _block_slots(1 if u == 0 else 0)
            for c in range(NC):
                pos = u * NC + c
                rel = scores[-2][0:8, 0:128] if len(scores) >= 2 else None
                hk = [[v_block(h, j, hp, par, k, lv, never,
                               lax.shift_right_logical(i + (u * NL + k // NPK), 16), rel)
                       for k in blocks.get((c, t), [])] for t in range(2)]
                l8, s = a_chunk(h, j, hp, par, c, l8, never, hk[0])
                prev = scores[-1] if scores else None
                scores.append(s)
                for q in KB_AT[j * NC + c]:
                    set_kb(1 - hp, h_k, q // 4, (q % 4) * (KV // 4), (q % 4 + 1) * (KV // 4),
                           never, prev)
                v0, v1 = KR_AT[j * NC + c]
                if v1 > v0:
                    set_kr(1 - hp, h_k, v0, v1)
                    kq = kr_bufs[1 - hp][pl.ds(_al(zero * 8), 8), :]
                    due.setdefault(pos + 2, []).append(pltpu.bitcast(kq, F32))
                dep = None
                for e in due.get(pos, []):
                    dep = e if dep is None else dep + e
                if KB_AT[j * NC + c]:
                    due.setdefault(pos + 2, []).append(
                        kb_bufs[1 - hp][pl.ds(_al(zero * 8), 8), :])
                pp = p_bufs[par][pl.ds(_al(zero * 8), 8), 0:128]
                n0 = (c % NL) * 128
                due.setdefault(pos + 2, []).extend([pltpu.bitcast(pp, F32), l8[:, n0:n0 + 128]])
                acc = b_chunk(h_b, 1 - par, B_ORDER[c], acc, zero, never,
                              hk[1] + ([] if dep is None else [dep]))
            ok = b_fin(h_b, (u - 1) % NQ, acc, l_prev, ok)
            l_prev = l8 + jnp.concatenate(lv, axis=1)
        return l_prev, acc, ok

    for cp in w_copies:
        cp.wait()
    ones = jnp.ones((8, TQ), F32)
    l_prev, _, ok = lax.fori_loop(0, H // HPB, body, (ones, jnp.zeros((DH, TQ), F32), ones))

    def pre(j, ln=True):
        r0, n = OS[j], OT[j]
        attn = lax.dot_general(_up(ot_s[r0 // TQ, :, r0 % TQ:r0 % TQ + n]), wo_v[...], TN,
                               preferred_element_type=F32)
        h = x_v[r0:r0 + n, :].astype(F32) + attn
        h_s[r0:r0 + n, :] = h
        if ln:
            hn_s[r0 // 2:(r0 + n) // 2, :] = _pk(_ln(h).astype(BF16))

    acc = jnp.zeros((DH, TQ), F32)
    for c in range(NC):
        acc = b_chunk(H - 1, 1, B_ORDER[c], acc, 0)
    ok = b_fin(H - 1, NQ - 1, acc, l_prev, ok)
    pre(0)
    pre(1, ln=False)

    @pl.when(jnp.min(ok) < 0.5)
    def _attention_with_row_max():
        def step(t, carry):
            h, j = t // NQ, t % NQ
            hrow = _al(h * 8)
            w_s[...] = jnp.zeros(w_s.shape, U32)
            w_s[pl.ds(_al((h % 8) * 8), 8), :] = qt_s[j, pl.ds(hrow, 8), :]
            s_s[...] = jnp.dot(_up(k_s[h // 8]), _up(w_s[...]), preferred_element_type=F32)
            m = jnp.max(s_s[...], axis=0, keepdims=True)
            p = jnp.exp2(s_s[...] - m)
            l = jnp.sum(p, axis=0, keepdims=True)
            o = jnp.dot(_up(vt_s[pl.ds(hrow, 8), :]), p.astype(BF16),
                        preferred_element_type=F32)
            ot_s[j, pl.ds(hrow, 8), :] = _pk((o / l).astype(BF16))
            return carry

        lax.fori_loop(0, H * NQ, step, 0)
        pre(0)
        pre(1, ln=False)

    def ffn(j):
        r0, n = OS[j], OT[j]
        hn = _up(hn_s[r0 // 2:(r0 + n) // 2, :])
        w_rem = jnp.concatenate([wg_v[FM:F, :], wu_v[FM:F, :]], axis=0)
        rem_t = lax.dot_general(w_rem, hn, NT, preferred_element_type=F32)
        a_rem_t = (_gelu_tanh(rem_t[0:F - FM]) * rem_t[F - FM:]).astype(BF16)
        gate = lax.dot_general(hn, wg_v[0:FM, :], NT, preferred_element_type=F32)
        up = lax.dot_general(hn, wu_v[0:FM, :], NT, preferred_element_type=F32)
        a = (_gelu_tanh(gate) * up).astype(BF16)
        y = (jnp.dot(a, wd_v[0:FM, :], preferred_element_type=F32)
             + lax.dot_general(a_rem_t, wd_v[FM:F, :], TN, preferred_element_type=F32))
        o_v[r0:r0 + n, :] = (h_s[r0:r0 + n, :] + y).astype(BF16)

    hn_s[OS[1] // 2:OS[2] // 2, :] = _pk(_ln(h_s[OS[1]:OS[2], :]).astype(BF16))
    for j in range(len(OT)):
        if j + 2 < len(OT):
            pre(j + 2)
        ffn(j)
        o_copy(j).start()
    for j in range(len(OT)):
        o_copy(j).wait()


def _call(x, wqkv, wo, wg_t, wu_t, wd, interpret=False):
    hbm = pl.BlockSpec(memory_space=pltpu.MemorySpace.HBM)
    return pl.pallas_call(
        _kernel,
        out_shape=jax.ShapeDtypeStruct((S, D), BF16),
        in_specs=[hbm] * 6,
        out_specs=hbm,
        scratch_shapes=[
            pltpu.VMEM((S, D), BF16),
            pltpu.VMEM((3, D, D), BF16),
            pltpu.VMEM((D, D), BF16),
            pltpu.VMEM((F, D), BF16),
            pltpu.VMEM((F, D), BF16),
            pltpu.VMEM((F, D), BF16),
            pltpu.VMEM((S, D), BF16),
            pltpu.VMEM((4, S // 2, 128), U32),
            pltpu.VMEM((NQ, D // 2, TQ), U32),
            pltpu.VMEM((D // 2, S), U32),
            pltpu.VMEM((NQ, D // 2, TQ), U32),
            pltpu.VMEM(((S - KV) // 2, TQ), U32),
            pltpu.VMEM(((S - KV) // 2, TQ), U32),
            pltpu.VMEM((KV // 2, TQ), U32),
            pltpu.VMEM((KV // 2, TQ), U32),
            pltpu.VMEM((64, TQ), U32),
            pltpu.VMEM(((S - KV) // 2, 128), U32),
            pltpu.VMEM(((S - KV) // 2, 128), U32),
            pltpu.VMEM((DH * KV, 128), F32),
            pltpu.VMEM((DH * KV, 128), F32),
            pltpu.VMEM((S, TQ), F32),
            pltpu.VMEM((S, D), F32),
            pltpu.VMEM((S // 2, D), U32),
            pltpu.SemaphoreType.DMA((len(XT),)),
            pltpu.SemaphoreType.DMA((7,)),
            pltpu.SemaphoreType.DMA((len(OT),)),
        ],
        compiler_params=pltpu.CompilerParams(vmem_limit_bytes=100 * 2 ** 20),
        interpret=interpret,
    )(x, wqkv, wo, wg_t, wu_t, wd)


@jax.jit
def pallas_sequential_preLN__softmax_full_mha__geglu_ffn__prompt_kernel(
    A_x: jax.Array,
    A_wqkv: jax.Array,
    A_wo: jax.Array,
    B_x: jax.Array,
    B_w_gate: jax.Array,
    B_w_up: jax.Array,
    B_w_down: jax.Array,
):
    out = _call(A_x.reshape(S, D), A_wqkv, A_wo, B_w_gate.T, B_w_up.T, B_w_down)
    return out.reshape(1, S, D)
```
